```python
import os as _os
_os.environ.setdefault("JAX_PLATFORMS", "cpu")
import jax
import jax.numpy as jnp

def _softmax(x, axis=-1):
    return jax.nn.softmax(x, axis=axis)
def _gelu(x):
    return jax.nn.gelu(x, approximate=True)
def _silu(x):
    return jax.nn.silu(x)
def _sigmoid(x):
    return jax.nn.sigmoid(x)
def _layernorm(x, axis=-1, eps=1e-5):
    m = jnp.mean(x, axis=axis, keepdims=True)
    v = jnp.var(x, axis=axis, keepdims=True)
    return (x - m) / jnp.sqrt(v + eps)
def _scatter_add(tgt, idx, src, axis=0):
    return tgt.at[idx].add(src)
def _segment_sum(src, seg, n):
    return jax.ops.segment_sum(src, seg, n)
class _Rng:
    def __init__(self, key):
        self._k = key
    def _next(self):
        self._k, sub = jax.random.split(self._k)
        return sub
    def normal(self, shape):
        return jax.random.normal(self._next(), shape, dtype=jnp.bfloat16)
    def randint(self, lo, hi, shape):
        return jax.random.randint(self._next(), shape, lo, hi, dtype=jnp.int32)
    def uniform(self, shape, lo=0.0, hi=1.0):
        return jax.random.uniform(self._next(), shape, jnp.bfloat16, lo, hi)
    def permutation(self, n):
        return jax.random.permutation(self._next(), n)


kernel_name = 'standalone__seq2seq_rnn_t_joint__speech'

def setup_inputs():
    _rng = _Rng(jax.random.key(int.from_bytes(__import__("os").urandom(4), "little")))
    _w = (lambda a: (lambda t: t.astype(jnp.bfloat16) if jnp.issubdtype(t.dtype, jnp.floating) else t)(jnp.asarray(a)))
    B, T, D, K = 2, 1000, 512, 31
    U = 8
    sc = (1.0 / (K * D)) ** 0.5
    sd = (1.0 / D) ** 0.5
    return {
        "x": _w((lambda *s: _rng.normal(s) * 0.4)(B, T, D) * 0.5),
        "w1": _w((lambda *s: _rng.normal(s) * 1.6)(K, D, D) * sc),
        "w2": _w((lambda *s: _rng.normal(s) * 1.6)(K, D, D) * sc),
        "g": _w((lambda *s: _rng.normal(s) * 1.6)(B, U, D) * 0.5),
        "w_f": _w((lambda *s: _rng.normal(s) * 1.6)(D, D) * sd),
        "w_g": _w((lambda *s: _rng.normal(s) * 1.6)(D, D) * sd),
        "w_o": _w((lambda *s: _rng.normal(s) * 1.6)(D, D) * sd),
    }

def reference(x, w1, w2, g, w_f, w_g, w_o):
    B, T, D = x.shape
    K = w1.shape[0]
    pad = K // 2
    xp = jnp.pad(x, ((0,0),(pad,pad),(0,0)))
    h = jnp.zeros_like(x)
    for i in range(K):
        h = h + jnp.einsum("btc,cd->btd", xp[:, i:i+T, :], w1[i])
    h = _gelu(h)[:, ::2, :]
    T1 = h.shape[1]
    hp = jnp.pad(h, ((0,0),(pad,pad),(0,0)))
    f = jnp.zeros_like(h)
    for i in range(K):
        f = f + jnp.einsum("btc,cd->btd", hp[:, i:i+T1, :], w2[i])
    f = _gelu(f)[:, ::2, :]
    fe = jnp.einsum("btd,de->bte", f, w_f)
    ge = jnp.einsum("bud,de->bue", g, w_g)
    j = jnp.tanh(fe[:, :, None, :] + ge[:, None, :, :])
    return jnp.einsum("btud,dv->btuv", j, w_o)
```

```python
import itertools

import jax
import jax.numpy as jnp
import jax.experimental.pallas as pl
import jax.experimental.pallas.tpu as pltpu

F32, BF16, U32 = jnp.float32, jnp.bfloat16, jnp.uint32
LANES = 128


def _sigmas(levels):
    return list(itertools.product(range(3), repeat=levels))


def _data_transform(z, levels):
    if levels == 0:
        return {(): z[0]}
    n = (len(z) - 1) // 2
    subs = (
        [z[2 * s + 1] for s in range(n)],
        [z[2 * s] - z[2 * s + 1] for s in range(n)],
        [z[2 * s + 2] - z[2 * s + 1] for s in range(n)],
    )
    out = {}
    for i, sub in enumerate(subs):
        for sig, v in _data_transform(sub, levels - 1).items():
            out[(i,) + sig] = v
    return out


def _weight_transform(w, levels):
    if levels == 0:
        return {(): w[0]}
    ev, od = w[0::2], w[1::2]
    both = [a if b is None else (b if a is None else a + b) for a, b in zip(ev, od)]
    out = {}
    for i, sub in enumerate((both, ev, od)):
        for sig, v in _weight_transform(sub, levels - 1).items():
            out[(i,) + sig] = v
    return out


def _raw_index(sig):
    if 0 in sig:
        return None
    return sum((i - 1) << l for l, i in enumerate(sig))


def _out_transform(y, levels):
    if levels == 0:
        return [y[()]]
    subs = [
        _out_transform({s[1:]: v for s, v in y.items() if s[0] == i}, levels - 1)
        for i in range(3)
    ]
    out = []
    for q in range(len(subs[0])):
        out += [subs[0][q] + subs[1][q], subs[0][q] + subs[2][q]]
    return out


def _interleave(main, side):
    n, m, done = len(main), len(side), 0
    for i, f in enumerate(main):
        f()
        upto = (m * (i + 1)) // n
        while done < upto:
            side[done]()
            done += 1


def _dot(a, b):
    return jnp.dot(a, b, preferred_element_type=F32)


def _kernel(x_hbm, w1_hbm, w2_hbm, g_hbm, wf_hbm, wg_hbm, wo_hbm, o_hbm,
            xs, w1s, w2s, gs, wfs, wgs, wos,
            d1, g1a, g1b, y1, a1, hs, d2, g2a, g2b, y2, fes, ges, outs,
            sem_x, sem_w1, sem_w2, sem_m, sem_o, *, T, K, U):
    B, NC = 2, 4
    T1, T2 = T // 2, T // 4
    S1, S2 = _sigmas(3), _sigmas(2)
    SUM1 = [s for s in S1 if _raw_index(s) is None]
    SUM2 = [s for s in S2 if _raw_index(s) is None]
    xs16 = xs.bitcast(BF16)

    def x_cp(b, k):
        return pltpu.make_async_copy(
            x_hbm.at[b, :, pl.ds(k * LANES, LANES)],
            xs16.at[b, k, pl.ds(16, T), :], sem_x.at[b, k])

    def w1_cp(j, c):
        n = min(16, K - 16 * c)
        return pltpu.make_async_copy(
            w1_hbm.at[pl.ds(16 * c, n), :, pl.ds(pl.multiple_of(j * LANES, LANES), LANES)],
            w1s.at[j, pl.ds(16 * c, n)], sem_w1.at[j, c])

    def w2_cp(k, ch):
        n = min(16, K - 16 * ch)
        return pltpu.make_async_copy(
            w2_hbm.at[pl.ds(16 * ch, n), pl.ds(pl.multiple_of(k * LANES, LANES), LANES), :],
            w2s.at[k, pl.ds(16 * ch, n)], sem_w2.at[k, ch])

    misc_cp = [pltpu.make_async_copy(s, d, sem_m.at[i]) for i, (s, d) in enumerate(
        ((g_hbm, gs), (wg_hbm, wgs), (wf_hbm, wfs), (wo_hbm, wos)))]

    tail0 = (16 + T) // 16 * 8
    for b in range(B):
        for k in range(NC):
            xs[b, k, pl.ds(0, 8), :] = jnp.zeros((8, LANES), U32)
            xs[b, k, pl.ds(tail0, xs.shape[2] - tail0), :] = jnp.zeros(
                (xs.shape[2] - tail0, LANES), U32)
    for k in range(NC):
        for b in range(B):
            x_cp(b, k).start()
    w1_cp(0, 0).start()
    w1_cp(0, 1).start()

    a1[...] = jnp.zeros_like(a1)
    y2[...] = jnp.zeros_like(y2)
    for r in range(8):
        for k in range(NC):
            hs[r, k, pl.ds(0, 16), :] = jnp.zeros((16, LANES), F32)
            hs[r, k, pl.ds(144, 16), :] = jnp.zeros((16, LANES), F32)

    def d1_chunk(k, carry):
        for b in range(B):
            x_cp(b, k).wait()

        def grp(gi, c2):
            v = [[xs[b, k, pl.ds(s + 64 * gi, 8, stride=8), :] for s in range(16)]
                 for b in range(B)]
            for eo in range(2):
                res = []
                for b in range(B):
                    z = [pltpu.unpack_elementwise(
                        v[b][s + eo], index=1 - eo, packed_dtype=BF16, unpacked_dtype=F32)
                        for s in range(15)]
                    res.append(_data_transform(z, 3))
                for si, sg in enumerate(S1):
                    w = pltpu.pack_elementwise([res[0][sg], res[1][sg]], packed_dtype=BF16)
                    d1[si, eo * NC + k, pl.ds(pl.multiple_of(gi * 8, 8), 8), :] = (
                        pltpu.bitcast(w, U32))
            return c2
        jax.lax.fori_loop(0, 9, grp, 0)
        return carry
    jax.lax.fori_loop(0, NC, d1_chunk, 0)

    def g1_prep(j, c, dst):
        def one(eo, rg):
            def f():
                rows = pl.ds(rg * 16, 16)
                w = []
                for s in range(8):
                    tap = 16 * c + 2 * s + eo
                    w.append(w1s[j, tap, rows, :].astype(F32) if tap < K else None)
                t = _weight_transform(w, 3)
                for i, sg in enumerate(SUM1):
                    dst[i, eo, rows, :] = t[sg].astype(BF16)
            return f
        return [one(eo, rg) for eo in range(2) for rg in range(32)]

    def mm1(j, c, src, sg):
        si = S1.index(sg)
        acc = None
        for eo in range(2):
            s = _raw_index(sg)
            if s is None:
                rhs = src[SUM1.index(sg), eo]
            else:
                tap = 16 * c + 2 * s + eo
                if tap >= K:
                    continue
                rhs = w1s[j, tap]
            lhs = jnp.concatenate(
                [pltpu.bitcast(d1[si, eo * NC + k, pl.ds(c, 64), :], BF16)
                 for k in range(NC)], axis=1)
            r = _dot(lhs, rhs)
            acc = r if acc is None else acc + r
        return acc

    def mm1_first(j):
        def one(sg):
            def f():
                y1[S1.index(sg)] = mm1(j, 0, g1a, sg)
            return f
        return [one(sg) for sg in S1]

    def mm1_second(j):
        def one(pi, p):
            def f():
                y = [y1[S1.index(p + (i,))] + mm1(j, 1, g1b, p + (i,)) for i in range(3)]
                a1[pi, 0] = y[0] + y[1]
                a1[pi, 1] = y[0] + y[2]
            return f
        return [one(pi, p) for pi, p in enumerate(S2)]

    def h_finish(k):
        def act(rg):
            def f():
                rows = pl.ds(rg * 8, 8)
                for top in range(2):
                    ph = _out_transform(
                        {p: a1[pi, top, rows, :] for pi, p in enumerate(S2)}, 2)
                    for q, v in enumerate(ph):
                        r = q + 4 * top
                        v = jax.nn.gelu(v, approximate=True)
                        nvalid = 2 * ((T1 - r + 7) // 8)
                        if nvalid < (rg + 1) * 8:
                            row = rg * 8 + jax.lax.broadcasted_iota(jnp.int32, v.shape, 0)
                            v = jnp.where(row < nvalid, v, 0.0)
                        hs[r, k, pl.ds(16 + rg * 8, 8), :] = v
            return f

        def dtr(eo, rg):
            def f():
                z = []
                for s in range(7):
                    ph = 2 * s + eo + 1
                    z.append(hs[ph % 8, k, pl.ds(12 + 2 * (ph // 8) + 16 * rg, 16), :])
                t = _data_transform(z, 2)
                for si, sg in enumerate(S2):
                    d2[si, eo * NC + k, pl.ds(rg * 8, 8), :] = pltpu.bitcast(
                        t[sg].astype(BF16), U32)
            return f
        return ([act(rg) for rg in range(16)]
                + [dtr(eo, rg) for rg in range(9) for eo in range(2)])

    w1_cp(0, 0).wait()
    for f in g1_prep(0, 0, g1a):
        f()

    def conv1_step(j, carry):
        @pl.when(j < NC - 1)
        def _():
            w1_cp(j + 1, 0).start()

        @pl.when(j >= 2)
        def _():
            w2_cp(2 * (j - 2), 0).start()
            w2_cp(2 * (j - 2), 1).start()

        w1_cp(j, 1).wait()
        _interleave(mm1_first(j), g1_prep(j, 1, g1b) + h_finish((j + NC - 1) % NC))

        @pl.when(j < NC - 1)
        def _():
            w1_cp(j + 1, 1).start()
            w1_cp(j + 1, 0).wait()

        @pl.when(j >= 2)
        def _():
            w2_cp(2 * (j - 2) + 1, 0).start()
            w2_cp(2 * (j - 2) + 1, 1).start()

        _interleave(mm1_second(j), g1_prep((j + 1) % NC, 0, g1a))
        return carry
    jax.lax.fori_loop(0, NC, conv1_step, 0)

    for cp in misc_cp:
        cp.start()

    def g2_prep(k, ch, dst):
        def one(cc, eo, rg):
            def f():
                rows = pl.ds(rg * 16, 16)
                w = []
                for s in range(4):
                    tap = 16 * ch + 8 * cc + 2 * s + eo
                    w.append(w2s[k, tap, rows, :].astype(F32) if tap < K else None)
                t = _weight_transform(w, 2)
                for i, sg in enumerate(SUM2):
                    dst[i, cc, eo, rows, :] = t[sg].astype(BF16)
            return f
        return [one(cc, eo, rg) for cc in range(2) for eo in range(2) for rg in range(8)]

    def mm2(k, ch, src):
        def one(si, sg):
            def f():
                lhs, rhs = [], []
                for cc in range(2):
                    for eo in range(2):
                        s = _raw_index(sg)
                        if s is None:
                            rhs.append(src[SUM2.index(sg), cc, eo])
                        else:
                            tap = 16 * ch + 8 * cc + 2 * s + eo
                            if tap >= K:
                                continue
                            rhs.append(w2s[k, tap])
                        lhs.append(pltpu.bitcast(
                            d2[si, eo * NC + k, pl.ds(2 * ch + cc, 64), :], BF16))
                y2[si] += _dot(jnp.concatenate(lhs, axis=1), jnp.concatenate(rhs, axis=0))
            return f
        return [one(si, sg) for si, sg in enumerate(S2)]

    for f in h_finish(NC - 1):
        f()
    w2_cp(0, 0).wait()
    for f in g2_prep(0, 0, g2a):
        f()

    def conv2_step(k, carry):
        w2_cp(k, 1).wait()
        _interleave(mm2(k, 0, g2a), g2_prep(k, 1, g2b))

        @pl.when(k < NC - 1)
        def _():
            w2_cp(k + 1, 0).wait()

        _interleave(mm2(k, 1, g2b), g2_prep((k + 1) % NC, 0, g2a))
        return carry
    jax.lax.fori_loop(0, NC, conv2_step, 0)

    for cp in misc_cp:
        cp.wait()
    gv = jnp.concatenate([gs[b] for b in range(B)], axis=0)
    ge = _dot(gv, wgs[...])
    for b in range(B):
        ges[b] = ge[b * U:(b + 1) * U]

    for hf in range(2):
        rows = pl.ds(hf * 64, 64)
        ph = _out_transform({sg: y2[si, rows, :] for si, sg in enumerate(S2)}, 2)
        fcat = jnp.concatenate(
            [jax.nn.gelu(v, approximate=True).astype(BF16) for v in ph], axis=0)
        fe = _dot(fcat, wfs[...])
        for r in range(4):
            for k in range(NC):
                fes[r, k, rows, :] = fe[r * 64:(r + 1) * 64, k * LANES:(k + 1) * LANES]

    TC = 64
    NCH = pl.cdiv(T2, TC)
    last = (T2 - (NCH - 1) * TC) * U

    def o_cp(b, ci, nrows):
        off = pl.multiple_of(ci * TC * U, TC * U)
        return pltpu.make_async_copy(
            outs.at[b, pl.ds(off, nrows), :], o_hbm.at[b, pl.ds(off, nrows), :],
            sem_o.at[b, ci])

    def joint_step(it, carry):
        b, ci = it // NCH, it % NCH
        gb = ges[b]
        cols = []
        for k in range(NC):
            gk = gb[:, k * LANES:(k + 1) * LANES]
            rows = []
            for t in range(TC):
                fr = fes[t % 4, k, pl.ds(2 * (ci * (TC // 4) + t // 4) + b, 1), :]
                rows.append(jnp.tanh(fr + gk))
            cols.append(jnp.concatenate(rows, axis=0).astype(BF16))
        res = _dot(jnp.concatenate(cols, axis=1), wos[...])
        outs[b, pl.ds(pl.multiple_of(ci * TC * U, TC * U), TC * U), :] = res.astype(BF16)

        @pl.when(ci < NCH - 1)
        def _():
            o_cp(b, ci, TC * U).start()

        @pl.when(ci == NCH - 1)
        def _():
            o_cp(b, ci, last).start()
        return carry
    jax.lax.fori_loop(0, B * NCH, joint_step, 0)

    for b in range(B):
        for ci in range(NCH):
            o_cp(b, ci, TC * U if ci < NCH - 1 else last).wait()


def _kernel_entry(*refs, T, K, U):
    return _kernel(*refs, T=T, K=K, U=U)


@jax.jit
def pallas_standalone__seq2seq_rnn_t_joint__speech_kernel(
    x: jax.Array,
    w1: jax.Array,
    w2: jax.Array,
    g: jax.Array,
    w_f: jax.Array,
    w_g: jax.Array,
    w_o: jax.Array,
):
    B, T, D = x.shape
    K, U = w1.shape[0], g.shape[1]
    assert (B, T, D, K, U) == (2, 1000, 512, 31, 8), "kernel is tiled for the task shapes"
    T2 = T // 4
    VM = pltpu.VMEM
    DMA = pltpu.SemaphoreType.DMA
    scratch = [
        VM((B, 4, 592, LANES), U32),
        VM((4, K, D, LANES), BF16),
        VM((4, K, LANES, D), BF16),
        VM((B, U, D), BF16),
        VM((D, D), BF16), VM((D, D), BF16), VM((D, D), BF16),
        VM((27, 8, 72, LANES), U32),
        VM((19, 2, D, LANES), BF16), VM((19, 2, D, LANES), BF16),
        VM((27, 128, LANES), F32),
        VM((9, 2, 128, LANES), F32),
        VM((8, 4, 160, LANES), F32),
        VM((9, 8, 72, LANES), U32),
        VM((5, 2, 2, LANES, D), BF16), VM((5, 2, 2, LANES, D), BF16),
        VM((9, 128, D), F32),
        VM((4, 4, 128, LANES), F32),
        VM((B, U, D), F32),
        VM((B, 256 * U, D), BF16),
        DMA((B, 4)), DMA((4, 2)), DMA((4, 2)), DMA((4,)), DMA((B, 4)),
    ]

    def body(*refs):
        _kernel(*refs, T=T, K=K, U=U)

    out = pl.pallas_call(
        body,
        out_shape=jax.ShapeDtypeStruct((B, T2 * U, D), BF16),
        in_specs=[pl.BlockSpec(memory_space=pl.ANY)] * 7,
        out_specs=pl.BlockSpec(memory_space=pl.ANY),
        scratch_shapes=scratch,
        compiler_params=pltpu.CompilerParams(vmem_limit_bytes=110 * 2**20),
    )(x, w1, w2, g, w_f, w_g, w_o)
    return out.reshape(B, T2, U, D)
```

```python
import itertools

import jax
import jax.numpy as jnp
import jax.experimental.pallas as pl
import jax.experimental.pallas.tpu as pltpu

F32, BF16, U32 = jnp.float32, jnp.bfloat16, jnp.uint32
LANES = 128
PC1, PC2, PC3 = 4, 4, 4
FPARTS = ((0, 32), (32, 48), (80, 48))
JCH = ((0, 64), (64, 64), (128, 64), (192, 40), (232, 18))


def _sigmas(levels):
    return list(itertools.product(range(3), repeat=levels))


def _data_transform(z, levels):
    if levels == 0:
        return {(): z[0]}
    n = (len(z) - 1) // 2
    subs = (
        [z[2 * s + 1] for s in range(n)],
        [z[2 * s] - z[2 * s + 1] for s in range(n)],
        [z[2 * s + 2] - z[2 * s + 1] for s in range(n)],
    )
    out = {}
    for i, sub in enumerate(subs):
        for sig, v in _data_transform(sub, levels - 1).items():
            out[(i,) + sig] = v
    return out


def _weight_transform(w, levels):
    if levels == 0:
        return {(): w[0]}
    ev, od = w[0::2], w[1::2]
    both = [a if b is None else (b if a is None else a + b) for a, b in zip(ev, od)]
    out = {}
    for i, sub in enumerate((both, ev, od)):
        for sig, v in _weight_transform(sub, levels - 1).items():
            out[(i,) + sig] = v
    return out


def _raw_index(sig):
    if 0 in sig:
        return None
    return sum((i - 1) << l for l, i in enumerate(sig))


def _out_transform(y, levels):
    if levels == 0:
        return [y[()]]
    subs = [
        _out_transform({s[1:]: v for s, v in y.items() if s[0] == i}, levels - 1)
        for i in range(3)
    ]
    out = []
    for q in range(len(subs[0])):
        out += [subs[0][q] + subs[1][q], subs[0][q] + subs[2][q]]
    return out


class _Feeder:
    def __init__(self, side, n):
        self.side, self.n, self.i, self.done = side, n, 0, 0

    def tick(self):
        self.i += 1
        upto = min(len(self.side), -(-len(self.side) * self.i // self.n))
        while self.done < upto:
            self.side[self.done]()
            self.done += 1


def _dot(a, b):
    return jnp.dot(a, b, preferred_element_type=F32)


def _kernel(x_hbm, w1_hbm, w2_hbm, g_hbm, wf_hbm, wg_hbm, wo_hbm, o_hbm,
            xs, w1s, w2s, gs, wfs, wgs, wos,
            d1, p1, q1, hs, p2, q2, fes, ges, outs, zs,
            sem_x, sem_w1, sem_w2, sem_m, sem_o, *, T, K, U):
    B, NC = 2, 4
    T1, T2 = T // 2, T // 4
    S1, S2 = _sigmas(3), _sigmas(2)
    SUM1 = [s for s in S1 if _raw_index(s) is None]
    SUM2 = [s for s in S2 if _raw_index(s) is None]
    xs16, w1s16, w2s16 = xs.bitcast(BF16), w1s.bitcast(BF16), w2s.bitcast(BF16)
    Y1 = 19 * 2 * 256
    D2 = Y1 + 27 * 128
    Y2 = 5 * 4 * NC * 64

    def put(buf, z, off, val):
        val = pltpu.bitcast(val, U32)
        buf[pl.ds(pl.multiple_of(z + off, 8), val.shape[0]), :] = val

    def put_fed(buf, z, off, val, feed, pieces):
        n = val.shape[0] // pieces
        for i in range(pieces):
            feed.tick()
            put(buf, z, off + i * n, val[i * n:(i + 1) * n])

    def getf(buf, off, n):
        return pltpu.bitcast(buf[pl.ds(off, n), :], F32)

    def getb(buf, off, n):
        return pltpu.bitcast(buf[pl.ds(off, n), :], BF16)

    def sums(words, levels, keys):
        halves = [_weight_transform(
            [None if w is None else pltpu.unpack_elementwise(
                w, index=i, packed_dtype=BF16, unpacked_dtype=F32) for w in words], levels)
            for i in range(2)]
        return [pltpu.pack_elementwise([halves[0][sg], halves[1][sg]], packed_dtype=BF16)
                for sg in keys]

    def x_cp(b, k):
        return pltpu.make_async_copy(
            x_hbm.at[b, :, pl.ds(k * LANES, LANES)],
            xs16.at[b, k, pl.ds(16, T), :], sem_x.at[b, k])

    def w1_cp(j, c):
        n = min(16, K - 16 * c)
        return pltpu.make_async_copy(
            w1_hbm.at[pl.ds(16 * c, n), :, pl.ds(pl.multiple_of(j * LANES, LANES), LANES)],
            w1s16.at[j, pl.ds(16 * c, n)], sem_w1.at[j, c])

    def w0_cp(k):
        return pltpu.make_async_copy(
            w1_hbm.at[pl.ds(0, 16), pl.ds(k * LANES, LANES), pl.ds(0, LANES)],
            w1s16.at[0, pl.ds(0, 16), pl.ds(k * LANES, LANES)], sem_x.at[2, k])

    def w2_cp(k, ch):
        n = min(16, K - 16 * ch)
        return pltpu.make_async_copy(
            w2_hbm.at[pl.ds(16 * ch, n), pl.ds(pl.multiple_of(k * LANES, LANES), LANES), :],
            w2s16.at[k, pl.ds(16 * ch, n)], sem_w2.at[k, ch])

    misc_cp = [pltpu.make_async_copy(s, d, sem_m.at[i]) for i, (s, d) in enumerate(
        ((g_hbm, gs), (wg_hbm, wgs), (wf_hbm, wfs), (wo_hbm, wos)))]

    tail0 = (16 + T) // 16 * 8
    for b in range(B):
        for k in range(NC):
            xs[b, k, pl.ds(0, 8), :] = jnp.zeros((8, LANES), U32)
            xs[b, k, pl.ds(tail0, xs.shape[2] - tail0), :] = jnp.zeros(
                (xs.shape[2] - tail0, LANES), U32)
    for k in range(2):
        for b in range(B):
            x_cp(b, k).start()
        w0_cp(k).start()
    p1[pl.ds(Y1, 27 * 128), :] = jnp.zeros((27 * 128, LANES), U32)

    zs[0] = 0
    zs[1] = 0
    for r in range(8):
        for k in range(NC):
            hs[r, k, pl.ds(0, 16), :] = jnp.zeros((16, LANES), F32)
            hs[r, k, pl.ds(144, 16), :] = jnp.zeros((16, LANES), F32)

    def d1_chunk(k, carry):
        for b in range(B):
            x_cp(b, k).wait()

        def grp(gi, c2):
            v = [[xs[b, k, pl.ds(s + 64 * gi, 8, stride=8), :] for s in range(16)]
                 for b in range(B)]
            for eo in range(2):
                res = []
                for b in range(B):
                    z = [pltpu.unpack_elementwise(
                        v[b][s + eo], index=1 - eo, packed_dtype=BF16, unpacked_dtype=F32)
                        for s in range(15)]
                    res.append(_data_transform(z, 3))
                for si, sg in enumerate(S1):
                    w = pltpu.pack_elementwise([res[0][sg], res[1][sg]], packed_dtype=BF16)
                    d1[si, eo * NC + k, pl.ds(pl.multiple_of(gi * 8, 8), 8), :] = (
                        pltpu.bitcast(w, U32))
            return c2
        jax.lax.fori_loop(0, 9, grp, 0)
        w0_cp(k).wait()

        @pl.when(k < 2)
        def _():
            for b in range(B):
                x_cp(b, k + 2).start()
            w0_cp(k + 2).start()

        pl.when(k == 1)(lambda: w1_cp(0, 1).start())
        pl.when(k == 2)(lambda: w1_cp(1, 0).start())
        pl.when(k == 3)(lambda: w1_cp(1, 1).start())
        row0 = pl.multiple_of(k * 64, 64)
        for eo in range(2):
            for rg in range(8):
                w = [w1s[0, 2 * s + eo, pl.ds(row0 + rg * 8, 8), :] for s in range(8)]
                for i, v in enumerate(sums(w, 3, SUM1)):
                    put(q1, 0, (2 * i + eo) * 64 + rg * 8, v)
        for si, sg in enumerate(S1):
            s = _raw_index(sg)
            lhs = [pltpu.bitcast(d1[si, eo * NC + k, pl.ds(0, 64), :], BF16) for eo in range(2)]
            rhs = [getb(q1, (2 * SUM1.index(sg) + eo) * 64, 64) if s is None else
                   pltpu.bitcast(w1s[0, 2 * s + eo, pl.ds(row0, 64), :], BF16)
                   for eo in range(2)]
            r = _dot(jnp.concatenate(lhs, axis=1), jnp.concatenate(rhs, axis=0))
            put(p1, 0, Y1 + si * 128, getf(p1, Y1 + si * 128, 128) + r)
        return carry
    jax.lax.fori_loop(0, NC, d1_chunk, 0)

    def g1_prep(j, c, dst, z):
        def one(eo, rg):
            def f():
                taps = [16 * c + 2 * s + eo for s in range(8)]
                w = [w1s[j, t, pl.ds(rg * 8, 8), :] if t < K else None for t in taps]
                for i, v in enumerate(sums(w, 3, SUM1)):
                    put(dst, z, (2 * i + eo) * 256 + rg * 8, v)
            return f
        return [one(eo, rg) for eo in range(2) for rg in range(32)]

    def mm1(j, c, src, sg):
        si = S1.index(sg)
        lhs, rhs = [], []
        for eo in range(2):
            s = _raw_index(sg)
            if s is None:
                rhs.append(getb(src, (2 * SUM1.index(sg) + eo) * 256, 256))
            else:
                tap = 16 * c + 2 * s + eo
                if tap >= K:
                    continue
                rhs.append(pltpu.bitcast(w1s[j, tap], BF16))
            lhs += [pltpu.bitcast(d1[si, eo * NC + k, pl.ds(c, 64), :], BF16)
                    for k in range(NC)]
        return _dot(jnp.concatenate(lhs, axis=1), jnp.concatenate(rhs, axis=0))

    def mm1_first(j, z, side):
        feed = _Feeder(side, 26 * PC1)
        for sg in S1:
            put_fed(p1, z, Y1 + S1.index(sg) * 128, mm1(j, 0, q1, sg), feed, PC1)

    def mm1_second(j, z, side):
        feed = _Feeder(side, 17 * PC2)
        for pi, p in enumerate(S2):
            for i in range(3):
                y = getf(p1, Y1 + S1.index(p + (i,)) * 128, 128) + mm1(j, 1, p1, p + (i,))
                if i == 0:
                    y0 = y
                else:
                    put_fed(q1, z, Y1 + (2 * pi + i - 1) * 128, y0 + y, feed, PC2)

    def h_finish(k, z):
        def act(rg):
            def f():
                for top in range(2):
                    ph = _out_transform(
                        {p: getf(q1, Y1 + (2 * pi + top) * 128 + rg * 8, 8)
                         for pi, p in enumerate(S2)}, 2)
                    for q, v in enumerate(ph):
                        r = q + 4 * top
                        v = jax.nn.gelu(v, approximate=True)
                        nvalid = 2 * ((T1 - r + 7) // 8)
                        if nvalid < (rg + 1) * 8:
                            row = rg * 8 + jax.lax.broadcasted_iota(jnp.int32, v.shape, 0)
                            v = jnp.where(row < nvalid, v, 0.0)
                        hs[r, k, pl.ds(16 + rg * 8, 8), :] = v
            return f

        def dtr(eo, rg):
            def f():
                zz = []
                for s in range(7):
                    ph = 2 * s + eo + 1
                    zz.append(hs[ph % 8, k, pl.ds(12 + 2 * (ph // 8) + 16 * rg, 16), :])
                t = _data_transform(zz, 2)
                for si, sg in enumerate(S2):
                    put(p1, z, D2 + (si * 8 + eo * NC + k) * 72 + rg * 8,
                        t[sg].astype(BF16))
            return f
        return ([act(rg) for rg in range(16)]
                + [dtr(eo, rg) for rg in range(9) for eo in range(2)])

    def g2_prep(k, ch, dst, z):
        def one(ce, rg, nk):
            def f():
                taps = [16 * ch + 8 * (ce // 2) + 2 * s + ce % 2 for s in range(4)]
                w = [w2s[k, t, pl.ds(rg * 8, 8), pl.ds(nk * LANES, LANES)] if t < K else None
                     for t in taps]
                for i, v in enumerate(sums(w, 2, SUM2)):
                    put(dst, z, ((i * 4 + ce) * NC + nk) * 64 + rg * 8, v)
            return f
        return [one(ce, rg, nk) for ce in range(4) for rg in range(8) for nk in range(NC)]

    w1_cp(0, 1).wait()
    for f in g1_prep(0, 1, p1, 0):
        f()

    def start_pair(cp, i):
        cp(i, 0).start()
        cp(i, 1).start()

    def conv1_step(j, carry):
        @pl.when(j > 0)
        def _():
            w1_cp(j, 1).wait()
            pl.when(j == 1)(lambda: start_pair(w1_cp, 3))
            pl.when(j >= 2)(lambda: start_pair(w2_cp, 2 * j - 3))
            mm1_first(j, zs[0], h_finish(j - 1, zs[1]) + g1_prep(j, 1, p1, zs[1]))

        pl.when(j == 0)(lambda: start_pair(w1_cp, 2))
        pl.when(j == 1)(lambda: start_pair(w2_cp, 0))
        pl.when(j == 2)(lambda: start_pair(w2_cp, 2))

        @pl.when(j < NC - 1)
        def _():
            w1_cp(j + 1, 0).wait()
            mm1_second(j, zs[0], g1_prep(j + 1, 0, q1, zs[1]))

        @pl.when(j == NC - 1)
        def _():
            for cp in misc_cp:
                cp.start()
            w2_cp(0, 0).wait()
            mm1_second(NC - 1, zs[0], g2_prep(0, 0, q1, zs[1]))
        return carry
    jax.lax.fori_loop(0, NC, conv1_step, 0)

    def mm2(k, ch, src, dst, acc, z, side):
        feed = _Feeder(side, 34 * PC3)
        for si, sg in enumerate(S2):
            lhs, rhs = [], []
            for ce in range(4):
                s = _raw_index(sg)
                if s is None:
                    base = (SUM2.index(sg) * 4 + ce) * NC
                    rhs.append(jnp.concatenate(
                        [getb(src, (base + nk) * 64, 64) for nk in range(NC)], axis=1))
                else:
                    tap = 16 * ch + 8 * (ce // 2) + 2 * s + ce % 2
                    if tap >= K:
                        continue
                    rhs.append(pltpu.bitcast(w2s[k, tap], BF16))
                lhs.append(getb(
                    p1, D2 + (si * 8 + (ce % 2) * NC + k) * 72 + 2 * ch + ce // 2, 64))
            r = _dot(jnp.concatenate(lhs, axis=1), jnp.concatenate(rhs, axis=0))
            for nk in range(NC):
                off = Y2 + (si * NC + nk) * 128
                v = r[:, nk * LANES:(nk + 1) * LANES]
                if acc is not None:
                    v = getf(acc, off, 128) + v
                put_fed(dst, z, off, v, feed, PC3)


    def conv2_step(k, carry):
        w2_cp(k, 1).wait()

        @pl.when(k == 0)
        def _():
            gp = g2_prep(0, 1, p2, zs[1])
            mm2(0, 0, q1, p2, None, zs[0], gp[:64] + h_finish(NC - 1, 0) + gp[64:])

        @pl.when(k > 0)
        def _():
            mm2(k, 0, q2, p2, q2, zs[0], g2_prep(k, 1, p2, zs[1]))

        @pl.when(k < NC - 1)
        def _():
            w2_cp(k + 1, 0).wait()

        mm2(k, 1, p2, q2, p2, zs[0], g2_prep((k + 1) % NC, 0, q2, zs[1]))
        return carry
    jax.lax.fori_loop(0, NC, conv2_step, 0)

    for cp in misc_cp:
        cp.wait()
    gv = jnp.concatenate([gs[b] for b in range(B)], axis=0)
    ge = _dot(gv, wgs[...])
    for b in range(B):
        ges[b] = ge[b * U:(b + 1) * U]

    for r0, nr in FPARTS:
        rows = pl.ds(r0, nr)
        ph = _out_transform(
            {sg: jnp.concatenate(
                [getf(q2, Y2 + (si * NC + nk) * 128 + r0, nr) for nk in range(NC)],
                axis=1) for si, sg in enumerate(S2)}, 2)
        fcat = jnp.concatenate(
            [jax.nn.gelu(v, approximate=True).astype(BF16) for v in ph], axis=0)
        fe = _dot(fcat, wfs[...])
        for r in range(4):
            for k in range(NC):
                fes[r, k, rows, :] = fe[r * nr:(r + 1) * nr, k * LANES:(k + 1) * LANES]

    def o_cp(b, ci):
        rows = pl.ds(JCH[ci][0] * U, JCH[ci][1] * U)
        return pltpu.make_async_copy(
            outs.at[b, rows, :], o_hbm.at[b, rows, :], sem_o.at[b, ci])

    def joint_chunk(b, t0, nt):
        gb = ges[b]
        cols = []
        for k in range(NC):
            gk = gb[:, k * LANES:(k + 1) * LANES]
            rows = []
            for t in range(nt):
                fr = fes[t % 4, k, pl.ds(2 * ((t0 + t) // 4) + b, 1), :]
                rows.append(jnp.tanh(fr + gk))
            cols.append(jnp.concatenate(rows, axis=0).astype(BF16))
        res = _dot(jnp.concatenate(cols, axis=1), wos[...])
        outs[b, pl.ds(t0 * U, nt * U), :] = res.astype(BF16)

    def joint_step(b, carry):
        for ci, (t0, nt) in enumerate(JCH):
            joint_chunk(b, t0, nt)
            o_cp(b, ci).start()
        return carry
    jax.lax.fori_loop(0, B, joint_step, 0)

    for b in range(B):
        for ci in range(len(JCH)):
            o_cp(b, ci).wait()


@jax.jit
def pallas_standalone__seq2seq_rnn_t_joint__speech_kernel(
    x: jax.Array,
    w1: jax.Array,
    w2: jax.Array,
    g: jax.Array,
    w_f: jax.Array,
    w_g: jax.Array,
    w_o: jax.Array,
):
    B, T, D = x.shape
    K, U = w1.shape[0], g.shape[1]
    assert (B, T, D, K, U) == (2, 1000, 512, 31, 8), "kernel is tiled for the task shapes"
    T2 = T // 4
    VM = pltpu.VMEM
    DMA = pltpu.SemaphoreType.DMA
    scratch = [
        VM((B, 4, 592, LANES), U32),
        VM((4, K, D // 2, LANES), U32),
        VM((4, K, LANES // 2, D), U32),
        VM((B, U, D), BF16),
        VM((D, D), BF16), VM((D, D), BF16), VM((D, D), BF16),
        VM((27, 8, 72, LANES), U32),
        VM((19 * 512 + 27 * 128 + 72 * 72, LANES), U32),
        VM((19 * 512 + 18 * 128, LANES), U32),
        VM((8, 4, 160, LANES), F32),
        VM((80 * 64 + 36 * 128, LANES), U32), VM((80 * 64 + 36 * 128, LANES), U32),
        VM((4, 4, 128, LANES), F32),
        VM((B, U, D), F32),
        VM((B, 256 * U, D), BF16),
        pltpu.SMEM((2,), jnp.int32),
        DMA((B + 1, 4)), DMA((4, 2)), DMA((4, 2)), DMA((4,)), DMA((B, len(JCH))),
    ]

    def body(*refs):
        _kernel(*refs, T=T, K=K, U=U)

    out = pl.pallas_call(
        body,
        out_shape=jax.ShapeDtypeStruct((B, T2 * U, D), BF16),
        in_specs=[pl.BlockSpec(memory_space=pl.ANY)] * 7,
        out_specs=pl.BlockSpec(memory_space=pl.ANY),
        scratch_shapes=scratch,
        compiler_params=pltpu.CompilerParams(vmem_limit_bytes=110 * 2**20),
    )(x, w1, w2, g, w_f, w_g, w_o)
    return out.reshape(B, T2, U, D)
```
